```python
import os as _os
_os.environ.setdefault("JAX_PLATFORMS", "cpu")
import jax
import jax.numpy as jnp

def _softmax(x, axis=-1):
    return jax.nn.softmax(x, axis=axis)
def _gelu(x):
    return jax.nn.gelu(x, approximate=True)
def _silu(x):
    return jax.nn.silu(x)
def _sigmoid(x):
    return jax.nn.sigmoid(x)
def _layernorm(x, axis=-1, eps=1e-5):
    m = jnp.mean(x, axis=axis, keepdims=True)
    v = jnp.var(x, axis=axis, keepdims=True)
    return (x - m) / jnp.sqrt(v + eps)
def _scatter_add(tgt, idx, src, axis=0):
    return tgt.at[idx].add(src)
def _segment_sum(src, seg, n):
    return jax.ops.segment_sum(src, seg, n)
class _Rng:
    def __init__(self, key):
        self._k = key
    def _next(self):
        self._k, sub = jax.random.split(self._k)
        return sub
    def normal(self, shape):
        return jax.random.normal(self._next(), shape, dtype=jnp.bfloat16)
    def randint(self, lo, hi, shape):
        return jax.random.randint(self._next(), shape, lo, hi, dtype=jnp.int32)
    def uniform(self, shape, lo=0.0, hi=1.0):
        return jax.random.uniform(self._next(), shape, jnp.bfloat16, lo, hi)
    def permutation(self, n):
        return jax.random.permutation(self._next(), n)


kernel_name = 'gated_mix__sliding_block__dense_activation_silu__prompt'

def setup_inputs():
    _rng = _Rng(jax.random.key(int.from_bytes(__import__("os").urandom(4), "little")))
    _w = (lambda a: (lambda t: t.astype(jnp.bfloat16) if jnp.issubdtype(t.dtype, jnp.floating) else t)(jnp.asarray(a)))
    def _A_setup():
        B, S, D = 1, 2048, 640
        return {
            "x": _w((lambda *s: _rng.normal(s) * 0.05)(B, S, D)),
            "wqkv": _w((lambda *s: _rng.normal(s) * 0.4)(D, 3 * D)),
            "wo": _w((lambda *s: _rng.normal(s) * 0.05)(D, D)),
        }
    _A_in = _A_setup()

    def _B_setup():
        B, S, D, F = 1, 2048, 640, 1536
        return {
            "x": _w((lambda *s: _rng.normal(s) * 0.05)(B, S, D)),
            "w1": _w((lambda *s: _rng.normal(s) * 1.6)(D, F) * (D ** -0.5)),
            "w2": _w((lambda *s: _rng.normal(s) * 1.6)(F, D) * (F ** -0.5)),
        }
    _B_in = _B_setup()

    return {
        "A_x": _A_in["x"],
        "A_wqkv": _A_in["wqkv"],
        "A_wo": _A_in["wo"],
        "B_x": _B_in["x"],
        "B_w1": _B_in["w1"],
        "B_w2": _B_in["w2"],
        "gate_w": _w((lambda *s: _rng.normal(s) * 0.05)(640) * 16.0),
    }

def reference(A_x, A_wqkv, A_wo, B_x, B_w1, B_w2, gate_w):
    def _A_ref(x, wqkv, wo):
        B, S, D = x.shape
        H = 32; Dh = D // H; W = 256
        qkv = (lambda x, *d: x.transpose(*d))((x @ wqkv).reshape(B, S, 3, H, Dh), 2, 0, 3, 1, 4)
        q, k, v = qkv[0], qkv[1], qkv[2]
        scores = jnp.einsum("bhqd,bhkd->bhqk", q, k) * (Dh ** -0.5)
        idx = jnp.arange(S)
        mask = (idx[:, None] - idx[None, :] >= 0) & (idx[:, None] - idx[None, :] < W)
        scores = jnp.where(mask[None, None], scores, -1e9)
        p = _softmax(scores, axis=-1)
        o = jnp.einsum("bhqk,bhkd->bhqd", p, v)
        return (lambda x, *d: x.transpose(*d))(o, 0, 2, 1, 3).reshape(B, S, D) @ wo

    def _B_ref(x, w1, w2):
        h = jnp.einsum("bsd,df->bsf", x, w1)
        h = _silu(h)
        out = jnp.einsum("bsf,fd->bsd", h, w2)
        return out

    x = A_x
    g = _sigmoid((x * gate_w).sum(-1, keepdims=True))
    a = _A_ref(x, A_wqkv, A_wo)
    b = _B_ref(x, B_w1, B_w2)
    return g * a + (1 - g) * b
```

```python
import functools
import math

import jax
import jax.numpy as jnp
import jax.experimental.pallas as pl
import jax.experimental.pallas.tpu as pltpu

S = 2048
D = 640
H = 32
DH = D // H
W = 256
F = 1536
TQ = 512
QB = 128
KW = W + QB
NEG = -1e9


def _kernel(x_ref, wqkv_ref, wo_ref, w1_ref, w2_ref, gw_ref, o_ref,
            wqvT_scr, k_scr, vT_scr, qT_scr, oT_scr):
    i = pl.program_id(0)
    f32, bf16 = jnp.float32, jnp.bfloat16

    @pl.when(i == 0)
    def _():
        wqvT_scr[0:D, :] = wqkv_ref[:, 0:D].astype(f32).T.astype(bf16)
        wqvT_scr[D:2 * D, :] = wqkv_ref[:, 2 * D:3 * D].astype(f32).T.astype(bf16)
        k_scr[0:W, :] = jnp.zeros((W, D), bf16)
        vT_scr[:, 0:W] = jnp.zeros((D, W), bf16)

    x = x_ref[...]
    r0 = pl.multiple_of(i * TQ, TQ)

    k = jnp.dot(x, wqkv_ref[:, D:2 * D], preferred_element_type=f32)
    k_scr[pl.ds(W + r0, TQ), :] = k.astype(bf16)
    qvT = jax.lax.dot_general(wqvT_scr[...], x, (((1,), (1,)), ((), ())),
                              preferred_element_type=f32)
    qT_scr[...] = qvT[0:D] * (DH ** -0.5 * math.log2(math.e))
    vT_scr[:, pl.ds(W + r0, TQ)] = qvT[D:2 * D].astype(bf16)

    ones = jnp.ones((16, KW), bf16)
    row128 = jax.lax.broadcasted_iota(jnp.int32, (128, QB), 0)
    row8 = jax.lax.broadcasted_iota(jnp.int32, (8, QB), 0)

    def qblock(b, carry):
        c0 = pl.multiple_of(b * QB, QB)
        q0 = pl.multiple_of(r0 + c0, QB)
        kpos = jax.lax.broadcasted_iota(jnp.int32, (KW, QB), 0) + (q0 - W)
        qpos = jax.lax.broadcasted_iota(jnp.int32, (KW, QB), 1) + q0
        diff = qpos - kpos
        valid = (diff >= 0) & (diff < W) & (kpos >= 0)
        bias = jnp.where(valid, 0.0, NEG).astype(f32)

        for g in range(H // 4):
            pieces = []
            for hh in range(4):
                h = 4 * g + hh
                lo = DH * h
                sT = None
                for t in sorted({lo // 128, (lo + DH - 1) // 128}):
                    qt = qT_scr[128 * t:128 * (t + 1), pl.ds(c0, QB)]
                    rows = row128 + 128 * t
                    qm = jnp.where((rows >= lo) & (rows < lo + DH), qt, 0.0).astype(bf16)
                    kt = k_scr[pl.ds(q0, KW), 128 * t:128 * (t + 1)]
                    part = jnp.dot(kt, qm, preferred_element_type=f32)
                    sT = part if sT is None else sT + part
                sT = sT + bias
                m = jnp.max(sT, axis=0, keepdims=True)
                p = jnp.exp2(sT - m).astype(bf16)
                w0 = 16 * (lo // 16)
                lhs = jnp.concatenate([vT_scr[w0:w0 + 32, pl.ds(q0, KW)], ones], axis=0)
                res = jnp.dot(lhs, p, preferred_element_type=f32)
                pieces.append(res[0:32] * (1.0 / res[32:33]))
            a, bb, c, d = pieces
            grp = jnp.concatenate([
                a[0:16],
                jnp.where(row8 < 4, a[16:24], bb[0:8]),
                bb[8:24],
                c[8:24],
                jnp.where(row8 < 4, c[24:32], d[8:16]),
                d[16:32],
            ], axis=0)
            oT_scr[80 * g:80 * (g + 1), pl.ds(c0, QB)] = grp
        return carry

    jax.lax.fori_loop(0, TQ // QB, qblock, 0)

    o = oT_scr[...].T.astype(bf16)
    att = jnp.dot(o, wo_ref[...], preferred_element_type=f32)

    hid = jnp.dot(x, w1_ref[...], preferred_element_type=f32)
    hid = (hid * jax.nn.sigmoid(hid)).astype(bf16)
    ffn = jnp.dot(hid, w2_ref[...], preferred_element_type=f32)

    logit = jnp.sum(x.astype(f32) * gw_ref[...].astype(f32), axis=-1, keepdims=True)
    g = jax.nn.sigmoid(logit)
    o_ref[...] = (g * att + (1.0 - g) * ffn).astype(o_ref.dtype)


@jax.jit
def pallas_gated_mix__sliding_block__dense_activation_silu__prompt_kernel(
    A_x: jax.Array,
    A_wqkv: jax.Array,
    A_wo: jax.Array,
    B_x: jax.Array,
    B_w1: jax.Array,
    B_w2: jax.Array,
    gate_w: jax.Array,
):
    del B_x
    x = A_x.reshape(S, D)
    gw = gate_w.reshape(1, D)
    const = lambda i: (0, 0)
    out = pl.pallas_call(
        _kernel,
        grid=(S // TQ,),
        in_specs=[
            pl.BlockSpec((TQ, D), lambda i: (i, 0)),
            pl.BlockSpec((D, 3 * D), const),
            pl.BlockSpec((D, D), const),
            pl.BlockSpec((D, F), const),
            pl.BlockSpec((F, D), const),
            pl.BlockSpec((1, D), const),
        ],
        out_specs=pl.BlockSpec((TQ, D), lambda i: (i, 0)),
        out_shape=jax.ShapeDtypeStruct((S, D), jnp.bfloat16),
        scratch_shapes=[
            pltpu.VMEM((2 * D, D), jnp.bfloat16),
            pltpu.VMEM((W + S, D), jnp.bfloat16),
            pltpu.VMEM((D, W + S), jnp.bfloat16),
            pltpu.VMEM((D, TQ), jnp.float32),
            pltpu.VMEM((D, TQ), jnp.float32),
        ],
        compiler_params=pltpu.CompilerParams(
            dimension_semantics=("arbitrary",),
            vmem_limit_bytes=100 * 1024 * 1024,
        ),
    )(x, A_wqkv, A_wo, B_w1, B_w2, gw)
    return out.reshape(1, S, D)
```

```python
import math

import jax
import jax.numpy as jnp
import jax.experimental.pallas as pl
import jax.experimental.pallas.tpu as pltpu

S = 2048
D = 640
H = 32
DH = D // H
W = 256
F = 1536
TQ = 512
QB = 128
HQ = QB // 2
KW = W + QB
KM = 2 * QB
NEG = -1e9
LOOKAHEAD = 3

_STRADDLE = [h for h in range(H) if (DH * h) // 128 != (DH * h + DH - 1) // 128]
_SLABS = [8 * ((DH * h) // 8) for h in _STRADDLE]
TILES = [[(h, 24 * j + DH * h - _SLABS[j]) for j, h in enumerate(_STRADDLE)]]
TILES += [[(h, DH * h - 128 * t) for h in range(H)
           if h not in _STRADDLE and (DH * h) // 128 == t] for t in range(D // 128)]
DK = D + 128


def _win(h):
    lo = DH * h
    w0 = 16 * (lo // 16)
    one_row = 0 if lo - w0 == 12 else 31
    return w0, one_row


def _kernel(x_ref, wqkv_hbm, wo_hbm, w1_hbm, w2_hbm, gw_ref, o_ref,
            wqkv_ref, wo_ref, w1_ref, w2_ref, sems,
            wqvT_scr, k_scr, vT_scr, qT_scr, oT_scr):
    i = pl.program_id(0)
    f32, bf16 = jnp.float32, jnp.bfloat16

    def wcopy(j):
        if j < 3:
            c = (1, 0, 2)[j]
            sl = (slice(None), slice(c * D, (c + 1) * D))
            return pltpu.make_async_copy(wqkv_hbm.at[sl], wqkv_ref.at[sl], sems.at[j])
        src, dst = ((wo_hbm, wo_ref), (w1_hbm, w1_ref), (w2_hbm, w2_ref))[j - 3]
        return pltpu.make_async_copy(src, dst, sems.at[j])

    @pl.when(i == 0)
    def _():
        for j in range(6):
            wcopy(j).start()
        k_scr[0:W, :] = jnp.zeros((W, DK), bf16)
        vT_scr[:, 0:W] = jnp.zeros((H * 32, W), bf16)
        wcopy(0).wait()

    x = x_ref[...]
    r0 = pl.multiple_of(i * TQ, TQ)

    k = jnp.dot(x, wqkv_ref[:, D:2 * D], preferred_element_type=f32)
    k_scr[pl.ds(W + r0, TQ), 0:D] = k.astype(bf16)

    @pl.when(i == 0)
    def _():
        wcopy(1).wait()
        wcopy(2).wait()
        wqvT_scr[0:D, :] = wqkv_ref[:, 0:D].astype(f32).T.astype(bf16)
        wqvT_scr[D:2 * D, :] = wqkv_ref[:, 2 * D:3 * D].astype(f32).T.astype(bf16)

    kb = k_scr[pl.ds(W + r0, TQ), 0:D].astype(f32)
    kx = jnp.concatenate([kb[:, s:s + 24] for s in _SLABS]
                         + [jnp.zeros((TQ, 128 - 24 * len(_SLABS)), f32)], axis=1)
    k_scr[pl.ds(W + r0, TQ), D:DK] = kx.astype(bf16)

    qvT = jax.lax.dot_general(wqvT_scr[...], x, (((1,), (1,)), ((), ())),
                              preferred_element_type=f32)
    qT_scr[...] = qvT[0:D] * (DH ** -0.5 * math.log2(math.e))
    row32 = jax.lax.broadcasted_iota(jnp.int32, (32, TQ), 0)
    for h in range(H):
        w0, one_row = _win(h)
        blk = jnp.where(row32 == one_row, 1.0, qvT[D + w0:D + w0 + 32])
        vT_scr[32 * h:32 * (h + 1), pl.ds(W + r0, TQ)] = blk.astype(bf16)

    rows = jax.lax.broadcasted_iota(jnp.int32, (128, QB), 0)
    row8 = jax.lax.broadcasted_iota(jnp.int32, (8, QB), 0)
    colA128 = jax.lax.broadcasted_iota(jnp.int32, (128, QB), 1) < HQ
    colA64 = jax.lax.broadcasted_iota(jnp.int32, (HQ, QB), 1) < HQ
    dim = jax.lax.broadcasted_iota(jnp.int32, (HQ, 128), 1)

    def make_bias(b):
        q0 = r0 + b * QB

        def mk(kpos):
            qpos = jax.lax.broadcasted_iota(jnp.int32, kpos.shape, 1) + q0
            diff = qpos - kpos
            valid = (diff >= 0) & (diff < W) & (kpos >= 0)
            return jnp.where(valid, 0.0, NEG).astype(f32)

        bm = mk(jax.lax.broadcasted_iota(jnp.int32, (KM, QB), 0) + (q0 - W + HQ))
        r = jax.lax.broadcasted_iota(jnp.int32, (HQ, QB), 0)
        bc = mk(jnp.where(colA64, r + (q0 - W), r + (q0 + HQ)))
        return bm, bc

    def qk_tile(b, t):
        q0 = pl.multiple_of(r0 + b * QB, QB)
        heads = TILES[t]
        cols = slice(b * QB, (b + 1) * QB)
        if t == 0:
            qt = jnp.concatenate([qT_scr[s:s + 24, cols] for s in _SLABS]
                                 + [jnp.zeros((128 - 24 * len(_SLABS), QB), f32)], axis=0)
            lanes = slice(D, DK)
        else:
            qt = qT_scr[128 * (t - 1):128 * t, cols]
            lanes = slice(128 * (t - 1), 128 * t)

        def sel(lo_a, lo_b):
            lo = lo_a if lo_a == lo_b else jnp.where(colA128, lo_a, lo_b)
            rel = rows - lo
            return jnp.where((rel >= 0) & (rel < DH), qt, 0.0).astype(bf16)

        qm = jnp.concatenate([sel(lo, lo) for _, lo in heads], axis=1)
        s_main = jnp.dot(k_scr[pl.ds(q0 + HQ, KM), lanes], qm, preferred_element_type=f32)

        none = (None, -4 * D)
        ev = [hl for hl in heads if hl[0] % 2 == 0]
        od = [hl for hl in heads if hl[0] % 2 == 1]
        n = max(len(ev), len(od))
        ev += [none] * (n - len(ev))
        od += [none] * (n - len(od))
        kf = k_scr[pl.ds(q0, HQ), lanes].astype(f32)
        kd = k_scr[pl.ds(q0 + W + HQ, HQ), lanes].astype(f32)
        par = jnp.zeros((HQ, 128), jnp.int32)
        for h, lo in heads:
            if h % 2 == 0:
                par = jnp.where((dim >= lo) & (dim < lo + DH), 1, par)
        even_lane = par > 0
        l1 = jnp.where(even_lane, kf, kd).astype(bf16)
        l2 = jnp.where(even_lane, kd, kf).astype(bf16)
        w1 = jnp.concatenate([sel(e[1], o[1]) for e, o in zip(ev, od)], axis=1)
        w2 = jnp.concatenate([sel(o[1], e[1]) for e, o in zip(ev, od)], axis=1)
        c1 = jnp.dot(l1, w1, preferred_element_type=f32)
        c2 = jnp.dot(l2, w2, preferred_element_type=f32)
        res = {}
        for j, (h, _) in enumerate(heads):
            res[h] = [s_main[:, 128 * j:128 * (j + 1)], None]
        for j, (e, o) in enumerate(zip(ev, od)):
            a1 = c1[:, 128 * j:128 * (j + 1)]
            a2 = c2[:, 128 * j:128 * (j + 1)]
            if e[0] is not None:
                res[e[0]][1] = jnp.where(colA64, a1, a2)
            if o[0] is not None:
                res[o[0]][1] = jnp.where(colA64, a2, a1)
        return res

    def head(b, h, sm, sc, bias):
        q0 = pl.multiple_of(r0 + b * QB, QB)
        bm, bc = bias

        def masked(y):
            if b == 0:
                return y + bm
            return jnp.concatenate(
                [y[0:HQ] + bm[0:HQ], y[HQ:HQ + QB], y[HQ + QB:] + bm[HQ + QB:]], axis=0)

        m = jnp.maximum(jnp.max(masked(sm), axis=0, keepdims=True),
                        jnp.max(sc + bc, axis=0, keepdims=True))
        pm = jnp.exp2(masked(sm - m))
        pc = jnp.exp2((sc - m) + bc)
        p = jnp.concatenate([jnp.where(colA64, pc, 0.0), pm, jnp.where(colA64, 0.0, pc)],
                            axis=0).astype(bf16)
        _, one_row = _win(h)
        lhs = vT_scr[32 * h:32 * (h + 1), pl.ds(q0, KW)]
        res = jnp.dot(lhs, p, preferred_element_type=f32)
        return res * (1.0 / res[one_row:one_row + 1])

    stages = [(b, t) for b in range(TQ // QB) for t in range(len(TILES))]
    outs = {}
    pend = [qk_tile(*stages[z]) for z in range(LOOKAHEAD)]
    bias = None
    for si, (b, t) in enumerate(stages):
        if si + LOOKAHEAD < len(stages):
            pend.append(qk_tile(*stages[si + LOOKAHEAD]))
        s_cur = pend.pop(0)
        if t == 0:
            bias = make_bias(b)
        for h, _ in TILES[t]:
            outs[h] = head(b, h, *s_cur[h], bias)
            g = h // 4
            if all(4 * g + e in outs for e in range(4)):
                a, bb, c, d = (outs.pop(4 * g + e) for e in range(4))
                grp = jnp.concatenate([
                    a[0:16],
                    jnp.where(row8 < 4, a[16:24], bb[0:8]),
                    bb[8:24],
                    c[8:24],
                    jnp.where(row8 < 4, c[24:32], d[8:16]),
                    d[16:32],
                ], axis=0)
                oT_scr[80 * g:80 * (g + 1), b * QB:(b + 1) * QB] = grp

    @pl.when(i == 0)
    def _():
        for j in range(3, 6):
            wcopy(j).wait()

    o = oT_scr[...].T.astype(bf16)
    att = jnp.dot(o, wo_ref[...], preferred_element_type=f32)

    hid = jnp.dot(x, w1_ref[...], preferred_element_type=f32)
    hid = (hid * jax.nn.sigmoid(hid)).astype(bf16)
    ffn = jnp.dot(hid, w2_ref[...], preferred_element_type=f32)

    logit = jnp.sum(x.astype(f32) * gw_ref[...].astype(f32).reshape(1, D), axis=-1, keepdims=True)
    g = jax.nn.sigmoid(logit)
    o_ref[...] = (g * att + (1.0 - g) * ffn).astype(o_ref.dtype)


@jax.jit
def pallas_gated_mix__sliding_block__dense_activation_silu__prompt_kernel(
    A_x: jax.Array,
    A_wqkv: jax.Array,
    A_wo: jax.Array,
    B_x: jax.Array,
    B_w1: jax.Array,
    B_w2: jax.Array,
    gate_w: jax.Array,
):
    del B_x
    x = A_x.reshape(S, D)
    hbm = pl.BlockSpec(memory_space=pl.ANY)
    out = pl.pallas_call(
        _kernel,
        grid=(S // TQ,),
        in_specs=[
            pl.BlockSpec((TQ, D), lambda i: (i, 0)),
            hbm, hbm, hbm, hbm,
            pl.BlockSpec((D,), lambda i: (0,)),
        ],
        out_specs=pl.BlockSpec((TQ, D), lambda i: (i, 0)),
        out_shape=jax.ShapeDtypeStruct((S, D), jnp.bfloat16),
        scratch_shapes=[
            pltpu.VMEM((D, 3 * D), jnp.bfloat16),
            pltpu.VMEM((D, D), jnp.bfloat16),
            pltpu.VMEM((D, F), jnp.bfloat16),
            pltpu.VMEM((F, D), jnp.bfloat16),
            pltpu.SemaphoreType.DMA((6,)),
            pltpu.VMEM((2 * D, D), jnp.bfloat16),
            pltpu.VMEM((W + S, DK), jnp.bfloat16),
            pltpu.VMEM((H * 32, W + S), jnp.bfloat16),
            pltpu.VMEM((D, TQ), jnp.float32),
            pltpu.VMEM((D, TQ), jnp.float32),
        ],
        compiler_params=pltpu.CompilerParams(
            dimension_semantics=("arbitrary",),
            vmem_limit_bytes=100 * 1024 * 1024,
        ),
    )(x, A_wqkv, A_wo, B_w1, B_w2, gate_w)
    return out.reshape(1, S, D)
```
